```python
import os as _os
_os.environ.setdefault("JAX_PLATFORMS", "cpu")
import jax
import jax.numpy as jnp

def _softmax(x, axis=-1):
    return jax.nn.softmax(x, axis=axis)
def _gelu(x):
    return jax.nn.gelu(x, approximate=True)
def _silu(x):
    return jax.nn.silu(x)
def _sigmoid(x):
    return jax.nn.sigmoid(x)
def _layernorm(x, axis=-1, eps=1e-5):
    m = jnp.mean(x, axis=axis, keepdims=True)
    v = jnp.var(x, axis=axis, keepdims=True)
    return (x - m) / jnp.sqrt(v + eps)
def _scatter_add(tgt, idx, src, axis=0):
    return tgt.at[idx].add(src)
def _segment_sum(src, seg, n):
    return jax.ops.segment_sum(src, seg, n)
class _Rng:
    def __init__(self, key):
        self._k = key
    def _next(self):
        self._k, sub = jax.random.split(self._k)
        return sub
    def normal(self, shape):
        return jax.random.normal(self._next(), shape, dtype=jnp.bfloat16)
    def randint(self, lo, hi, shape):
        return jax.random.randint(self._next(), shape, lo, hi, dtype=jnp.int32)
    def uniform(self, shape, lo=0.0, hi=1.0):
        return jax.random.uniform(self._next(), shape, jnp.bfloat16, lo, hi)
    def permutation(self, n):
        return jax.random.permutation(self._next(), n)


kernel_name = 'parallel_sum__sliding_local_dilated__geglu_ffn__prompt'

def setup_inputs():
    _rng = _Rng(jax.random.key(int.from_bytes(__import__("os").urandom(4), "little")))
    _w = (lambda a: (lambda t: t.astype(jnp.bfloat16) if jnp.issubdtype(t.dtype, jnp.floating) else t)(jnp.asarray(a)))
    def _A_setup():
        B, S, D = 1, 2048, 640
        return {
            "x": _w((lambda *s: _rng.normal(s) * 0.05)(B, S, D)),
            "wqkv": _w((lambda *s: _rng.normal(s) * 0.05)(D, 3 * D)),
            "wo": _w((lambda *s: _rng.normal(s) * 0.05)(D, D)),
        }
    _A_in = _A_setup()

    def _B_setup():
        B, S, D, F = 1, 2048, 640, 1728
        return {
            "x": _w((lambda *s: _rng.normal(s) * 0.05)(B, S, D)),
            "w_gate": _w((lambda *s: _rng.normal(s) * 0.05)(D, F)),
            "w_up": _w((lambda *s: _rng.normal(s) * 0.05)(D, F)),
            "w_down": _w((lambda *s: _rng.normal(s) * 0.05)(F, D)),
        }
    _B_in = _B_setup()

    return {
        "A_x": _A_in["x"],
        "A_wqkv": _A_in["wqkv"],
        "A_wo": _A_in["wo"],
        "B_x": _B_in["x"],
        "B_w_gate": _B_in["w_gate"],
        "B_w_up": _B_in["w_up"],
        "B_w_down": _B_in["w_down"],
    }

def reference(A_x, A_wqkv, A_wo, B_x, B_w_gate, B_w_up, B_w_down):
    def _A_ref(x, wqkv, wo):
        B, S, D = x.shape
        H = 32; Dh = D // H
        W, dil = 8, 2
        qkv = (lambda x, *d: x.transpose(*d))((x @ wqkv).reshape(B, S, 3, H, Dh), 2, 0, 3, 1, 4)
        q, k, v = qkv[0], qkv[1], qkv[2]
        scale = Dh ** -0.5
        pos = jnp.arange(S)
        off = jnp.arange(W) * dil
        idx = pos[:, None] - off[None, :]
        mask = idx >= 0
        idx_c = jnp.where(mask, idx, 0).reshape(-1)
        kg = k[:, :, idx_c, :].reshape(B, H, S, W, Dh)
        vg = v[:, :, idx_c, :].reshape(B, H, S, W, Dh)
        logits = jnp.einsum("bhsd,bhswd->bhsw", q, kg) * scale
        logits = jnp.where(mask[None, None, :, :], logits, -1e9)
        attn = _softmax(logits, axis=-1)
        o = jnp.einsum("bhsw,bhswd->bhsd", attn, vg)
        return (lambda x, *d: x.transpose(*d))(o, 0, 2, 1, 3).reshape(B, S, D) @ wo

    def _B_ref(x, w_gate, w_up, w_down):
        return (_gelu(x @ w_gate) * (x @ w_up)) @ w_down

    x = A_x
    xn = _layernorm(x, axis=-1)
    return x + _A_ref(xn, A_wqkv, A_wo) + _B_ref(xn, B_w_gate, B_w_up, B_w_down)
```

```python
import functools
import math
import jax
import jax.numpy as jnp
from jax import lax
import jax.experimental.pallas as pl
import jax.experimental.pallas.tpu as pltpu

_H, _W, _DIL = 32, 8, 2
_HALO = 16
_L = 128
_F32, _BF16, _U32 = jnp.float32, jnp.bfloat16, jnp.uint32


def _gelu(x):
    c = math.sqrt(2.0 / math.pi)
    hx = 0.5 * x
    return hx + hx * jnp.tanh(x * (c + (c * 0.044715) * (x * x)))


def _lhs7(a11, a12, a21, a22):
    return (a11 + a22, a21 + a22, a11, a22, a11 + a12, a21 - a11, a12 - a22)


def _rhs7(b11, b12, b21, b22):
    return (b11 + b22, b11, b12 - b22, b21 - b11, b22, b11 + b12, b21 + b22)


def _put(ref, idx, r0, v):
    ref[idx + (pl.ds(r0, v.shape[0]),)] = v.astype(_BF16)
    return v[-8:].astype(_F32)


def _get(ref, idx, r0=0, n=_L):
    return ref.bitcast(_U32)[idx + (pl.ds(r0 // 2, n // 2),)]


class _Pacer:
    def __init__(self, true):
        self.true, self.now, self.jobs, self.done = true, 0, [], []

    def spread(self, jobs, t0, t1, slack=None):
        self.jobs += [(self.now + t0 + (t1 - t0) * i // len(jobs), slack, job) for i, job in enumerate(jobs)]
        self.jobs.sort(key=lambda e: e[0])

    def run(self, after, upto):
        while self.jobs and self.jobs[0][0] <= upto:
            _, slack, job = self.jobs.pop(0)
            out = job(after)
            if slack is not None:
                self.done.append((self.now + slack, out))

    def dot(self, lhs, rhs, transposed):
        late = [v for t, v in self.done if t <= self.now]
        self.done = [(t, v) for t, v in self.done if t > self.now]
        if late:
            head = functools.reduce(lambda u, v: jnp.where(self.true, u, pltpu.bitcast(v, _U32)), late, lhs[0][:8])
            lhs = [jnp.concatenate([head, lhs[0][8:]], axis=0)] + lhs[1:]
        a, b = (pltpu.bitcast(jnp.concatenate(v, axis=1), _BF16) for v in (lhs, rhs))
        r = lax.dot_general(a, b, (((1,), (int(transposed),)), ((), ())), preferred_element_type=_F32)
        self.now += a.shape[0] * len(lhs) * r.shape[1] // (4 * _L)
        tok = r[:8, :_L]

        def after(v):
            reps = (v.shape[0] // 8, v.shape[1] // _L)
            return jnp.where(jnp.tile(self.true, reps), v, jnp.tile(tok, reps))

        self.run(after, self.now)
        return r


def _impl(A_x, A_wqkv, A_wo, B_x, B_w_gate, B_w_up, B_w_down, tm0=512, tm=256, ar=8, lr=16, la=2, roll3=1,
          order0="012hABCV345", order="ABCVh012345", dg=2, dpos=(5, 6, 7, 10), qpos=(2, 3, 5), nx=2, la0=3, midp=5,
          at1=80, at0=50, asl=600, lt0=(25, 36), lt1=(0, 35), lsl=500, pw=3, waits=(0, 1, 2, 3, 5, 7, 10), wfirst=2, unroll=1, ylast=0, flags=None):
    del B_x
    _, S, D = A_x.shape
    F = B_w_gate.shape[1]
    Dh = D // _H
    ND = D // _L
    NF = F // _L
    FR = F - NF * _L
    nb = (S - tm0) // tm
    tmx = max(tm0, tm)
    c_exp = Dh ** -0.5 * math.log2(math.e)
    tile = lambda i, n=1: pl.ds(i * _L, n * _L)
    lt = lambda v, j: v[:, j * _L:(j + 1) * _L]
    rows = lambda *parts: jnp.concatenate(parts, axis=0)
    total = lambda parts: functools.reduce(jnp.add, parts)
    same = lambda v: v
    pairs = ([(("g", c), ("u", c)) for c in range(NF)] + [(("q", j), ("k", j)) for j in range(ND)]
             + [(("v", 4), ("t", 0)), (("v", 0), ("v", 1)), (("v", 2), ("v", 3))])
    kpairs = ([(("h", c), ("h", c + 1)) for c in range(0, NF - 1, 2)]
              + [(("h", NF - 1), ("o", 0)), (("o", 1), ("o", 2)), (("o", 3), ("o", 4))])
    NP, NK = len(pairs), len(kpairs)
    stages = {str(i): (2 * i, 2) for i in range(NF // 2)}
    stages.update(h=(NF - 1, 1), A=(NF, 2), B=(NF + 2, 2), C=(NF + 4, 2), V=(NF + 6, 2), a=(0, 1), b=(1, 1))

    def kernel(x_hbm, wqkv_hbm, wo_hbm, wg_hbm, wu_hbm, wd_hbm, o_hbm,
               x_s, o_s, wqkv_raw, wo_raw, wg_raw, wu_raw, wd_raw, tr, w1, w2, wt,
               xa, xp, q_s, k_s, v_s, att, h12, ha, ht, zero, i_sem, o_sem):
        n_sem = [0]

        def cp(src, dst):
            n_sem[0] += 1
            return pltpu.make_async_copy(src, dst, i_sem.at[n_sem[0] - 1])

        def out_cp(i, part, row, n):
            r = pl.ds(pl.multiple_of(row, 16), n), tile(4, 1) if part else tile(0, 4)
            return pltpu.make_async_copy(o_s.at[r], o_hbm.at[0].at[r], o_sem.at[2 * i + part])

        def w_rows(kind, t, e):
            if kind in "qkvo":
                return [tr["qkvo".index(kind)][j, pl.ds(4 * t + e, _H, stride=Dh), :] for j in range(ND)]
            if kind == "t":
                ref, r0 = (wg_raw, wu_raw)[e * _H // FR], NF * _L + e * _H % FR
            else:
                ref, r0 = dict(g=wg_raw, u=wu_raw, h=wd_raw)[kind], t * _L + e * _H
            return [ref[pl.ds(r0, _H), tile(j)].astype(_F32) for j in range(ND)]

        def prep1(p, e, after):
            left, right = (w_rows(*t, e) for t in pairs[p])
            for k in range(2):
                for i, b in enumerate(_rhs7(left[k], right[k], left[2 + k], right[2 + k])):
                    _put(w1[p], (2 * i + k,), e * _H, b)
            _put(w1[p], (14,), e * _H, left[4])
            _put(w1[p], (15,), e * _H, right[4])

        def prep2(p, e, after):
            first, second = (w_rows(*t, e) for t in kpairs[p])
            for k in range(2):
                for i, b in enumerate(_rhs7(after(first[k]), first[2 + k], second[k], after(second[2 + k]))):
                    out = _put(w2[p], (2 * i + k,), e * _H, b)
            _put(w2[p], (14,), e * _H, first[4])
            _put(w2[p], (15,), e * _H, second[4])
            return out

        def widen_wo(j, after):
            tr[3][j] = wo_raw[:, tile(j)].astype(_F32)
            _put(wt, (j,), FR, jnp.zeros((_L - FR, _L), _F32))
            return _put(wt, (j,), 0, wd_raw[pl.ds(NF * _L, FR), tile(j)])

        def transpose_qkv(s, j, after):
            tr[s][j] = wqkv_raw[s, tile(j), :].astype(_F32).T

        def layernorm(row, hm, r, n, after):
            xn = []
            for half in range(2):
                x = after(x_s[pl.ds(pl.multiple_of(row + half * hm + r, 16), n), :].astype(_F32))
                xc = x - jnp.mean(x, axis=-1, keepdims=True)
                var = jnp.mean(xc * xc, axis=-1, keepdims=True)
                xn.append(xc * lax.rsqrt(var + 1e-5))
                _put(xp, (), half * hm + r, lt(xn[half], 4))
            for k in range(2):
                for i, a in enumerate(_lhs7(*[lt(xn[half], j) for half in range(2) for j in (k, 2 + k)])):
                    out = _put(xa, (i, k), r, a)
            return out

        def proj(pc, c, n, hm, mid):
            a = lambda i: [_get(xa, (i, k), 0, hm) for k in range(2)]
            b = lambda i, j, n: [rows(*[_get(w1[c + j + t], (2 * i + k,)) for t in range(n)]) for k in range(2)]
            m = [pc.dot(a(i), b(i, 0, n), True) for i in range(midp)]
            mid()
            m += [pc.dot(a(i), b(i, 0, n), True) for i in range(midp, 5)]
            out = []
            for j in range(n):
                e = [lt(v, j) for v in m]
                top, bot = [_get(xp, (), 0, hm)], [_get(xp, (), hm, hm)]
                bl, br = [_get(w1[c + j], (14,))], [_get(w1[c + j], (15,))]
                c11 = pc.dot(a(6) + top, b(6, j, 1) + bl, True) + (e[0] + e[3] - e[4])
                c12 = pc.dot(top, br, True) + (e[2] + e[4])
                c22 = pc.dot(a(5) + bot, b(5, j, 1) + br, True) + (e[0] - e[1] + e[2])
                c21 = pc.dot(bot, bl, True) + (e[1] + e[3])
                out.append([c11, c12, c21, c22])
            return out

        def put_h(p, r0, a11, a12, a21, a22):
            return [_put(ha, (i, p), r0, a) for i, a in enumerate(_lhs7(a11, a12, a21, a22) + (a12, a21))][0]

        def attention(r0, first, after):
            back = lambda ref, j, w: ref[j, pl.ds(r0 + _HALO - _DIL * w, ar), :]
            q = [after(q_s[j, pl.ds(r0, ar), :]) for j in range(ND)]
            lg = []
            for w in range(_W):
                a = total([q[j] * back(k_s, j, w) for j in range(ND)])
                if roll3:
                    a = (a + pltpu.roll(a, 64, 1)) + (pltpu.roll(a, 32, 1) + pltpu.roll(a, 96, 1))
                else:
                    a = a + pltpu.roll(a, 64, 1)
                    a = a + pltpu.roll(a, 32, 1)
                if first and r0 < _DIL * w:
                    pos = r0 + lax.broadcasted_iota(jnp.int32, a.shape, 0)
                    a = jnp.where(pos >= _DIL * w, a, -1e9 * Dh ** 0.5)
                lg.append(a)
            m = functools.reduce(jnp.maximum, lg)
            p = [jnp.exp2((a - m) * c_exp) for a in lg]
            inv = 1.0 / total(p)
            for j in range(ND):
                o = inv * total([p[w] * back(v_s, j, w) for w in range(_W)])
                att[j, pl.ds(r0, ar), :] = o
            return o[-8:]

        def pack_attention(r, n, hm, after):
            t = lambda i, r0: (att.at[i - 1] if i else h12)[pl.ds(r0, n), :]
            return [put_h(NF // 2 + i // 2, r, t(i, r), t(i + 1, r), t(i, hm + r), t(i + 1, hm + r))
                    for i in range(0, ND + 1, 2)][-1]

        def stage(pc, name, hm, mid=tuple):
            c, n = stages[name]
            res = proj(pc, c, n, hm, mid)
            if c < NF:
                h = [(_gelu(gt) * ut, _gelu(gb) * ub) for gt, ut, gb, ub in res]
                if c % 2:
                    h = [(att[0, pl.ds(0, hm), :], att[0, pl.ds(hm, hm), :])] + h
                if len(h) == 2:
                    put_h(c // 2, 0, h[0][0], h[1][0], h[0][1], h[1][1])
                else:
                    (h12 if name == "h" else att.at[0])[pl.ds(0, 2 * hm), :] = rows(*h[0])
                return
            for pair, quad in zip(pairs[c:c + n], res):
                for side, (kind, j) in enumerate(pair):
                    r = rows(*quad[side::2])
                    if kind == "t":
                        lane = lax.broadcasted_iota(jnp.int32, r.shape, 1)
                        _put(ht, (), 0, jnp.where(lane < FR, _gelu(r) * pltpu.roll(r, FR, 1), 0.0))
                    else:
                        dict(q=q_s, k=k_s, v=v_s)[kind][j, pl.ds(0 if kind == "q" else _HALO, 2 * hm), :] = r

        def down(pc, row, hm, sem0, between):
            a = lambda i, ps: [_get(ha, (i, p), 0, hm) for p in ps]
            b = lambda i, ps: [rows(*[_get(w2[p], (2 * i + k,)) for p in ps]) for k in range(2)]
            bt = lambda j: [_get(wt, (j,)), _get(wt, (j + 1,))]
            a5 = lambda ps: [rows(*a(i, [p]), *a(j, [p])) for p in ps for i, j in ((2, 8), (7, 3))]
            b5 = lambda ps: [_get(w2[p], (k,)) for p in ps for k in (14, 15)]
            top, bot = _get(ht, (), 0, hm), _get(ht, (), hm, hm)

            def emit(half, j, y):
                r = pl.ds(pl.multiple_of(row + half * hm, 16), y.shape[0]), pl.ds(j * _L, y.shape[1])
                o_s[r] = (x_s[r].astype(_F32) + y).astype(o_s.dtype)

            groups = [range(p, p + dg) for p in range(0, NF // 2, dg)]
            m = [total([pc.dot(a(i, ps), b(i, ps), False) for ps in groups]) for i in range(7)]
            y = [pc.dot(a5(ps), [rows(*b5(ps))], False) for ps in groups[ylast:]]
            between()
            ps = range(NF // 2, NK)
            m[:5] = [m[i] + pc.dot(a(i, ps), b(i, ps), False) for i in range(5)]
            emit(0, 2, pc.dot([top], bt(2), False) + (m[2] + m[4]))
            emit(1, 0, pc.dot([bot], bt(0), False) + (m[1] + m[3]))
            emit(0, 0, pc.dot(a(6, ps) + [top], list(map(rows, b(6, ps), bt(0))), False) + (m[0] + m[3] - m[4] + m[6]))
            emit(1, 2, pc.dot(a(5, ps) + [bot], list(map(rows, b(5, ps), bt(2))), False) + (m[0] - m[1] + m[2] + m[5]))
            out_cp(sem0, 0, row, 2 * hm).start()
            y = total(y + [pc.dot(a5(ps), [rows(*b5(ps))], False) for ps in groups[:ylast]])
            emit(0, 4, pc.dot(a5(ps) + [rows(top, bot)], [rows(*b5(ps), _get(wt, (4,)))], False) + y)
            out_cp(sem0, 1, row, 2 * hm).start()

        def block(row, sem0, hm, next_row, names, hooks=None):
            pc = _Pacer(zero[...] == 0)
            for i, name in enumerate(names):
                stage(pc, name, hm, functools.partial(hooks[i], pc) if hooks else tuple)
                if name == "h" and "V" in names[:i]:
                    assert sum(job.func is pack_attention for _, _, job in pc.jobs) == hm // max(ar, 16)
                if name == "V":
                    jobs, n = [], max(ar, 16)
                    for r in range(0, hm, n):
                        jobs += [functools.partial(attention, half * hm + r + s, bool(hooks))
                                 for half in range(2) for s in range(0, n, ar)]
                        jobs.append(functools.partial(pack_attention, r, n, hm))
                    pc.spread(jobs, 0, (at0 if hooks else at1) * hm, asl)
            t0, t1 = lt0 if hooks else lt1
            pc.spread([functools.partial(layernorm, next_row, tm // 2, r, lr) for r in range(0, tm // 2, lr)],
                      t0 * hm, t1 * hm, lsl)

            def between():
                assert all(job.func is layernorm for _, _, job in pc.jobs)
                k_s[:, pl.ds(0, _HALO), :] = k_s[:, pl.ds(2 * hm, _HALO), :]
                v_s[:, pl.ds(0, _HALO), :] = v_s[:, pl.ds(2 * hm, _HALO), :]

            down(pc, row, hm, sem0, between)
            assert not pc.jobs

        feed = [([], [], []) for _ in range(nx + len(order0) + 1)]
        rows_cp = lambda src, dst, r0, n: cp(src.at[pl.ds(r0, n)], dst.at[pl.ds(r0, n)])
        job = functools.partial
        wait_at = lambda i: feed[nx + max(j for j in waits if j <= i)][0]
        xr = tm0 // 2 // nx
        for i in range(nx):
            feed[i + (i >= wfirst)][0].extend(rows_cp(x_hbm.at[0], x_s, half * tm0 // 2 + i * xr, xr) for half in range(2))
            feed[i + (i >= wfirst)][1].append(job(layernorm, 0, tm0 // 2, i * xr, xr))
        for s in range(3):
            wait_at(qpos[s]).append(cp(wqkv_hbm.at[:, pl.ds(s * D, D)], wqkv_raw.at[s]))
            feed[nx + qpos[s]][1].extend(job(transpose_qkv, s, j) for j in range(ND))
        for i, name in enumerate(order0):
            c, n = stages[name]
            if c < NF or name == "C":
                r0, nr = (c * _L, n * _L) if c < NF else (NF * _L, FR)
                (wait_at(i) if i else feed[wfirst][0]).extend(
                    [rows_cp(wg_hbm, wg_raw, r0, nr), rows_cp(wu_hbm, wu_raw, r0, nr)])
            feed[nx + i if i else wfirst][1].extend(job(prep1, p, e) for p in range(c, c + n) for e in range(4))
        for i, (lo, hi) in zip(dpos, ((0, 2), (2, 4), (4, 6), (6, NK))):
            wait_at(i).append(rows_cp(wd_hbm, wd_raw, 2 * lo * _L, min(F, 2 * hi * _L) - 2 * lo * _L))
            if hi == NK:
                wait_at(i).extend([cp(wo_hbm, wo_raw), rows_cp(x_hbm.at[0], x_s, tm0, tm)])
                feed[nx + i][2].extend(job(widen_wo, j) for j in range(ND))
            feed[nx + i][2].extend(job(prep2, p, e) for p in range(lo, hi) for e in range(4))
        rest = rows_cp(x_hbm.at[0], x_s, tm0 + tm, S - tm0 - tm)
        started = [0]

        def start(upto):
            for copies, _, _ in feed[started[0]:upto]:
                for c in copies:
                    c.start()
            started[0] = max(started[0], upto)

        def consume(i, pc=None):
            for c in feed[i][0]:
                c.wait()
            if feed[i][0]:
                nxt = [j for j in range(i + 1, len(feed)) if feed[j][0]][:la]
                start(nxt[-1] + 1) if nxt else rest.start()
            for work in feed[i][1]:
                work(same)
            if feed[i][2]:
                pc.spread(feed[i][2], pw * tm0 // 2, 8 * tm0 // 2, tm0)

        start(la0)
        zero[...] = jnp.zeros(zero.shape, zero.dtype)
        k_s[:, pl.ds(0, _HALO), :] = jnp.zeros((ND, _HALO, _L), _F32)
        v_s[:, pl.ds(0, _HALO), :] = jnp.zeros((ND, _HALO, _L), _F32)
        for i in range(nx + 1):
            consume(i)
        block(0, 0, tm0 // 2, tm0, order0, [functools.partial(consume, i) for i in range(nx + 1, len(feed))])
        rest.wait()

        @pl.loop(0, nb, unroll=unroll)
        def _(b):
            row = tm0 + b * tm
            block(row, b + 1, tm // 2, jnp.minimum(row + tm, S - tm), order)

        for part in range(2):
            out_cp(0, part, 0, tm0).wait()
            for b in range(nb):
                out_cp(b + 1, part, tm0 + b * tm, tm).wait()

    vm = pltpu.VMEM
    packed = lambda *shape: vm(shape + (_L,), _BF16)
    return pl.pallas_call(
        kernel,
        in_specs=[pl.BlockSpec(memory_space=pl.ANY)] * 6,
        out_specs=pl.BlockSpec(memory_space=pl.ANY),
        out_shape=jax.ShapeDtypeStruct(A_x.shape, A_x.dtype),
        scratch_shapes=[
            vm((S, D), A_x.dtype), vm((S, D), A_x.dtype), vm((3, D, D), _BF16), vm((D, D), _BF16),
            vm((F, D), _BF16), vm((F, D), _BF16), vm((F, D), _BF16), [vm((ND, D, _L), _F32)] * 4,
            [packed(16, _L)] * NP, [packed(16, _L)] * NK, packed(ND, _L),
            packed(7, 2, tmx // 2), packed(tmx),
            vm((ND, tmx, _L), _F32), vm((ND, tmx + _HALO, _L), _F32), vm((ND, tmx + _HALO, _L), _F32),
            vm((ND, tmx, _L), _F32), vm((tmx, _L), _F32), packed(9, NK, tmx // 2), packed(tmx),
            vm((8, _L), jnp.int32), pltpu.SemaphoreType.DMA((40,)), pltpu.SemaphoreType.DMA((2 * nb + 2,)),
        ],
        compiler_params=pltpu.CompilerParams(vmem_limit_bytes=100 * 1024 * 1024, flags=flags),
    )(A_x, A_wqkv, A_wo, B_w_gate.T, B_w_up.T, B_w_down)


@jax.jit
def pallas_parallel_sum__sliding_local_dilated__geglu_ffn__prompt_kernel(A_x, A_wqkv, A_wo, B_x, B_w_gate, B_w_up, B_w_down):
    return _impl(A_x, A_wqkv, A_wo, B_x, B_w_gate, B_w_up, B_w_down)
```

```python
import functools
import math

import jax
import jax.numpy as jnp
from jax import lax
import jax.experimental.pallas as pl
import jax.experimental.pallas.tpu as pltpu

_H, _W, _DIL = 32, 8, 2
_HALO = 16
_L = 128
_F32, _BF16, _U32 = jnp.float32, jnp.bfloat16, jnp.uint32


def _gelu(x):
    c = math.sqrt(2.0 / math.pi)
    hx = 0.5 * x
    return hx + hx * jnp.tanh(x * (c + (c * 0.044715) * (x * x)))


def _lhs7(a11, a12, a21, a22):
    return (a11 + a22, a21 + a22, a11, a22, a11 + a12, a21 - a11, a12 - a22)


def _rhs7(b11, b12, b21, b22):
    return (b11 + b22, b11, b12 - b22, b21 - b11, b22, b11 + b12, b21 + b22)


def _put(ref, idx, r0, v):
    ref[idx + (pl.ds(r0, v.shape[0]),)] = v.astype(_BF16)
    return v[-8:].astype(_F32)


def _get(ref, idx, r0=0, n=_L):
    return ref.bitcast(_U32)[idx + (pl.ds(r0 // 2, n // 2),)]


class _Pacer:
    def __init__(self, always):
        self.always, self.now, self.jobs, self.done = always, 0, [], []

    def spread(self, jobs, t0, t1, slack):
        self.jobs += [(self.now + t0 + (t1 - t0) * i // len(jobs), slack, job) for i, job in enumerate(jobs)]
        self.jobs.sort(key=lambda e: e[0])

    def pending(self, fn):
        return sum(job.func is fn for _, _, job in self.jobs)

    def dot(self, lhs, rhs, rhs_transposed):
        due = [v for t, v in self.done if t <= self.now]
        self.done = [(t, v) for t, v in self.done if t > self.now]
        if due:
            head = functools.reduce(lambda u, v: jnp.where(self.always, u, pltpu.bitcast(v, _U32)), due, lhs[0][:8])
            lhs = [jnp.concatenate([head, lhs[0][8:]], axis=0)] + lhs[1:]
        a, b = (pltpu.bitcast(jnp.concatenate(v, axis=1), _BF16) for v in (lhs, rhs))
        r = lax.dot_general(a, b, (((1,), (int(rhs_transposed),)), ((), ())), preferred_element_type=_F32)
        self.now += a.shape[0] * len(lhs) * r.shape[1] // (4 * _L)

        def after(v):
            reps = (v.shape[0] // 8, v.shape[1] // _L)
            return jnp.where(jnp.tile(self.always, reps), v, jnp.tile(r[:8, :_L], reps))

        while self.jobs and self.jobs[0][0] <= self.now:
            _, slack, job = self.jobs.pop(0)
            self.done.append((self.now + slack, job(after)))
        return r


def _impl(A_x, A_wqkv, A_wo, B_x, B_w_gate, B_w_up, B_w_down, order0="01hABCV2345", order="ABCVh012345",
          qpos=(2, 3, 4), dpos=(6, 6, 8, 10), waits=(0, 1, 2, 3, 4, 6, 8, 10), at=(61, 78), nt=((26, 39), (26, 39)),
          st=36, pw=24, asl=600, lsl=500, nsl=300, halves=True, la=3, mseq=(0, 1, 2, 3, 4), dg=2,
          dseq=(0, 3, 4, 2, 1, 6, 5, 7, 8), interpret=False):
    del B_x
    _, S, D = A_x.shape
    F = B_w_gate.shape[1]
    tm0, tm = 512, 256
    nb = (S - tm0) // tm
    Dh = D // _H
    ND, NF = D // _L, F // _L
    FR = F - NF * _L
    assert (ND, NF, FR) == (5, 13, 64) and S == tm0 + nb * tm and nb > 1
    c_exp = Dh ** -0.5 * math.log2(math.e)
    job = functools.partial
    tile = lambda i, n=1: pl.ds(i * _L, n * _L)
    lt = lambda v, j: v[:, j * _L:(j + 1) * _L]
    rows = lambda *parts: jnp.concatenate(parts, axis=0)
    total = lambda parts: functools.reduce(jnp.add, parts)
    qkv = [(kind, j) for kind in "qkv" for j in range(ND)] + [("t", 0)]
    pairs = [(("g", c), ("u", c)) for c in range(NF)] + list(zip(qkv[::2], qkv[1::2]))
    w2_tiles = [("h", c) for c in range(NF)] + [("o", j) for j in range(ND)]
    kpairs = list(zip(w2_tiles[::2], w2_tiles[1::2]))
    NK = len(kpairs)
    stages = {str(i): (2 * i, 2) for i in range(NF // 2)}
    stages.update(h=(NF - 1, 1), A=(NF, 2), B=(NF + 2, 2), C=(NF + 4, 2), V=(NF + 6, 2))

    def kernel(x_hbm, wqkv_hbm, wo_hbm, wg_hbm, wu_hbm, wd_hbm, o_hbm,
               x_s, o_s, wqkv_raw, wo_raw, wg_raw, wu_raw, wd_raw, wide, w1, w2, wt,
               stat, xa, q_s, k_s, v_s, att, h_last, ha, ht, zero, i_sem, o_sem):
        def out_copy(part, row, hm):
            r = pl.ds(pl.multiple_of(row + min(part, 1) * hm, 16), hm), (tile(0, 5), tile(0, 4), tile(4))[part]
            return pltpu.make_async_copy(o_s.at[r], o_hbm.at[0].at[r], o_sem)

        def w_rows(kind, t, e):
            if kind in "qkvo":
                return [wide["qkvo".index(kind)][j, pl.ds(4 * t + e, _H, stride=Dh), :] for j in range(ND)]
            if kind == "t":
                ref, r0 = (wg_raw, wu_raw)[e * _H // FR], NF * _L + e * _H % FR
            else:
                ref, r0 = dict(g=wg_raw, u=wu_raw, h=wd_raw)[kind], t * _L + e * _H
            return [ref[pl.ds(r0, _H), tile(j)].astype(_F32) for j in range(ND)]

        def prep_w1(p, e):
            left, right = (w_rows(*t, e) for t in pairs[p])
            for k in range(2):
                for i, b in enumerate(_rhs7(left[k], right[k], left[2 + k], right[2 + k]) + ((left, right)[k][4],)):
                    _put(w1[p], (2 * i + k,), e * _H, b)

        def prep_w2(p, e, after):
            first, second = (w_rows(*t, e) for t in kpairs[p])
            for k in range(2):
                _put(w2[p], (14 + k,), e * _H, (first, second)[k][4])
                for i, b in enumerate(_rhs7(after(first[k]), first[2 + k], second[k], after(second[2 + k]))):
                    out = _put(w2[p], (2 * i + k,), e * _H, b)
            return out

        def widen_wo(j, after):
            wide[3][j] = wo_raw[:, tile(j)].astype(_F32)
            _put(wt, (j,), FR, jnp.zeros((_L - FR, _L), _F32))
            return _put(wt, (j,), 0, wd_raw[pl.ds(NF * _L, FR), tile(j)])

        def transpose_qkv(s, j):
            wide[s][j] = wqkv_raw[s, tile(j), :].astype(_F32).T

        def row_stats(row, r, n, after=lambda v: v):
            x = after(x_s[pl.ds(pl.multiple_of(row + r, 16), n), :].astype(_F32))
            mean = jnp.mean(x, axis=-1, keepdims=True)
            xc = x - mean
            scale = jnp.broadcast_to(lax.rsqrt(jnp.mean(xc * xc, axis=-1, keepdims=True) + 1e-5), (n, _L))
            stat[0, pl.ds(r, n), :] = jnp.broadcast_to(mean, (n, _L))
            stat[1, pl.ds(r, n), :] = scale
            return scale[-8:]

        def normalize(row, hm, r, n, after=lambda v: v):
            xn = []
            for r0 in (r, hm + r):
                mean, scale = after(stat[0, pl.ds(r0, n), :]), stat[1, pl.ds(r0, n), :]
                x = x_s[pl.ds(pl.multiple_of(row + r0, 16), n), :].astype(_F32)
                xn.append([(lt(x, j) - mean) * scale for j in range(ND)])
            for k in range(2):
                _put(xa, (14 + k,), r, xn[k][4])
                for i, a in enumerate(_lhs7(xn[0][k], xn[0][2 + k], xn[1][k], xn[1][2 + k])):
                    out = _put(xa, (2 * i + k,), r, a)
            return out

        def project(pc, c, n, r0, nr, midway):
            a = lambda i: [_get(xa, (2 * i + k,), r0, nr) for k in range(2)]
            b = lambda i, ps: [rows(*[_get(w1[p], (2 * i + k,)) for p in ps]) for k in range(2)]
            m = {i: pc.dot(a(i), b(i, range(c, c + n)), True) for i in mseq}
            midway(pc)
            out = []
            for p in range(c, c + n):
                e = [lt(m[i], p - c) for i in range(5)]
                (top, bot), (left, right) = a(7), b(7, [p])
                c11 = pc.dot(a(6) + [top], b(6, [p]) + [left], True) + (e[0] + e[3] - e[4])
                c12 = pc.dot([top], [right], True) + (e[2] + e[4])
                c22 = pc.dot(a(5) + [bot], b(5, [p]) + [right], True) + (e[0] - e[1] + e[2])
                c21 = pc.dot([bot], [left], True) + (e[1] + e[3])
                out.append((c11, c12, c21, c22))
            return out

        def put_h(p, r0, a11, a12, a21, a22):
            return [_put(ha, (i, p), r0, a) for i, a in enumerate(_lhs7(a11, a12, a21, a22) + (a12, a21))][0]

        def stage(pc, name, r0, nr, midway):
            c, n = stages[name]
            res = project(pc, c, n, r0, nr, midway)
            if c < NF:
                h = [(_gelu(gt) * ut, _gelu(gb) * ub) for gt, ut, gb, ub in res]
                if n == 2:
                    put_h(c // 2, r0, h[0][0], h[1][0], h[0][1], h[1][1])
                else:
                    h_last[pl.ds(0, 2 * nr), :] = rows(*h[0])
                return
            for pair, quad in zip(pairs[c:c + n], res):
                for side, (kind, j) in enumerate(pair):
                    r = rows(*quad[side::2])
                    if kind == "t":
                        lane = lax.broadcasted_iota(jnp.int32, r.shape, 1)
                        _put(ht, (), 0, jnp.where(lane < FR, _gelu(r) * pltpu.roll(r, FR, 1), 0.0))
                    else:
                        dict(q=q_s, k=k_s, v=v_s)[kind][j, pl.ds(0 if kind == "q" else _HALO, 2 * nr), :] = r

        def attention(r0, first, after):
            back = lambda ref, j, w: ref[j, pl.ds(r0 + _HALO - _DIL * w, 8), :]
            q = [after(q_s[j, pl.ds(r0, 8), :]) for j in range(ND)]
            logits = []
            for w in range(_W):
                a = total([q[j] * back(k_s, j, w) for j in range(ND)])
                a = (a + pltpu.roll(a, 2 * _H, 1)) + (pltpu.roll(a, _H, 1) + pltpu.roll(a, 3 * _H, 1))
                if first and r0 < _DIL * w:
                    pos = r0 + lax.broadcasted_iota(jnp.int32, a.shape, 0)
                    a = jnp.where(pos >= _DIL * w, a, -1e9 * Dh ** 0.5)
                logits.append(a)
            m = functools.reduce(jnp.maximum, logits)
            p = [jnp.exp2((a - m) * c_exp) for a in logits]
            inv = 1.0 / total(p)
            for j in range(ND):
                o = inv * total([p[w] * back(v_s, j, w) for w in range(_W)])
                att[j, pl.ds(r0, 8), :] = o
            return o

        def pack_attention(r, hm, after):
            t = lambda i, r0: att[i - 1, pl.ds(r0, 16), :] if i else h_last[pl.ds(r0, 16), :]
            return [put_h(NF // 2 + i // 2, r, t(i, r), t(i + 1, r), t(i, hm + r), t(i + 1, hm + r))
                    for i in range(0, ND + 1, 2)][-1]

        def output(pc, row, hm):
            a = lambda i, ps: [_get(ha, (i, p), 0, hm) for p in ps]
            bt = lambda j, n: [_get(wt, (j + k,)) for k in range(n)]
            top, bot = _get(ht, (), 0, hm), _get(ht, (), hm, hm)

            def emit(half, j, y):
                r = pl.ds(pl.multiple_of(row + half * hm, 16), hm), pl.ds(j * _L, y.shape[1])
                o_s[r] = (x_s[r].astype(_F32) + y).astype(o_s.dtype)

            def product(i, ps, extra=()):
                if i < 7:
                    lhs, rhs = a(i, ps), [rows(*[_get(w2[p], (2 * i + k,)) for p in ps]) for k in range(2)]
                else:
                    lhs = [v for p in ps for j in ((2, 7), (8, 3))[i - 7] for v in a(j, [p])]
                    rhs = [rows(*[_get(w2[p], (k,)) for p in ps for k in (14, 15)])]
                if extra:
                    lhs, rhs = lhs + [extra[0]], list(map(rows, rhs, extra[1]))
                return pc.dot(lhs, rhs, False)

            ffn = {i: [product(i, range(p, p + dg)) for p in range(0, NF // 2, dg)] for i in dseq}
            assert len(pc.jobs) == pc.pending(row_stats) + pc.pending(normalize)
            k_s[:, pl.ds(0, _HALO), :] = k_s[:, pl.ds(2 * hm, _HALO), :]
            v_s[:, pl.ds(0, _HALO), :] = v_s[:, pl.ds(2 * hm, _HALO), :]
            full = lambda i, *extra: total(ffn[i] + [product(i, range(NF // 2, NK), extra)])
            m = {i: full(i) for i in dseq if i < 5}
            emit(0, 2, pc.dot([top], bt(2, 2), False) + (m[2] + m[4]))
            emit(0, 0, full(6, top, bt(0, 2)) + (m[0] + m[3] - m[4]))
            emit(0, 4, full(7, top, bt(4, 1)))
            out_copy(0, row, hm).start()
            emit(1, 0, pc.dot([bot], bt(0, 2), False) + (m[1] + m[3]))
            emit(1, 2, full(5, bot, bt(2, 2)) + (m[0] - m[1] + m[2]))
            out_copy(1, row, hm).start()
            emit(1, 4, full(8, bot, bt(4, 1)))
            out_copy(2, row, hm).start()

        def block(row, hm, next_row, names, hooks=None):
            first = hooks is not None
            pc = _Pacer(zero[...] == 0)
            stats = [job(row_stats, next_row, r, 16) for r in range(0, tm, 16)]
            if not first:
                pc.spread(stats, 0, st * hm, lsl)
            for i, name in enumerate(names):
                nr = hm // 2 if first and halves and i == 0 else hm
                for r0 in range(0, hm, nr):
                    stage(pc, name, r0, nr, hooks.pop(0) if first else lambda pc: None)
                if name == "V":
                    if first:
                        k_s[:, pl.ds(0, _HALO), :] = jnp.zeros((ND, _HALO, _L), _F32)
                        for j in range(ND):
                            v_s[j, pl.ds(0, _HALO), :] = jnp.broadcast_to(v_s[j, pl.ds(_HALO, 1), :], (_HALO, _L))
                    jobs = []
                    for r in range(0, hm, 16):
                        jobs += [job(attention, r + s, first) for s in (0, 8, hm, hm + 8)]
                        jobs.append(job(pack_attention, r, hm))
                    pc.spread(jobs, 0, at[not first] * hm, asl)
                if name == "h" and "V" in names[:i]:
                    assert pc.pending(pack_attention) == hm // 16
            t0, t1 = nt[not first]
            if first:
                pc.spread(stats, 0, t0 * hm, lsl)
            pc.spread([job(normalize, next_row, tm // 2, r, 16) for r in range(0, tm // 2, 16)], t0 * hm, t1 * hm, nsl)
            output(pc, row, hm)
            assert not pc.jobs

        feed = [([], [], []) for _ in range(len(order0) + 3)]
        by_rows = lambda src, dst, r0, n: (src.at[pl.ds(r0, n)], dst.at[pl.ds(r0, n)])
        wait_at = lambda i: feed[2 + max(j for j in waits if j <= i)][0]
        hm0, xr = tm0 // 2, tm0 // 4
        for i in range(2):
            feed[i][0].extend(by_rows(x_hbm.at[0], x_s, r0, xr) for r0 in (i * xr, hm0 + i * xr))
            feed[i][1].extend([job(row_stats, 0, i * xr, xr), job(row_stats, 0, hm0 + i * xr, xr),
                               job(normalize, 0, hm0, i * xr, xr)])
        for s in range(3):
            wait_at(qpos[s]).append((wqkv_hbm.at[:, pl.ds(s * D, D)], wqkv_raw.at[s]))
            feed[2 + qpos[s]][1].extend(job(transpose_qkv, s, j) for j in range(ND))
        for i, name in enumerate(order0):
            c, n = stages[name]
            if c < NF or name == "V":
                r0, nr = (c * _L, n * _L) if c < NF else (NF * _L, FR)
                wait_at(i).extend([by_rows(wg_hbm, wg_raw, r0, nr), by_rows(wu_hbm, wu_raw, r0, nr)])
            feed[2 + i][1].extend(job(prep_w1, p, e) for p in range(c, c + n) for e in range(4))
        for i, (lo, hi) in zip(dpos, ((0, 2), (2, 4), (4, 6), (6, NK))):
            wait_at(i).append(by_rows(wd_hbm, wd_raw, 2 * lo * _L, min(F, 2 * hi * _L) - 2 * lo * _L))
            if hi == NK:
                wait_at(i).extend([(wo_hbm, wo_raw), by_rows(x_hbm.at[0], x_s, tm0, tm)])
                feed[2 + i][2].extend(job(widen_wo, j) for j in range(ND))
            feed[2 + i][2].extend(job(prep_w2, p, e) for p in range(lo, hi) for e in range(4))
        feed.append(([by_rows(x_hbm.at[0], x_s, tm0 + tm, S - tm0 - tm)], [], []))
        if halves:
            feed[1:3] = feed[2], feed[1]
        queue = [f[0] for f in feed if f[0]]
        for i, group in enumerate(queue):
            group[:] = [pltpu.make_async_copy(src, dst, i_sem.at[i % 3]) for src, dst in group]
        in_flight = []

        def refill(n):
            while queue and len(in_flight) < (n if len(queue) > 1 else 1):
                in_flight.append(queue.pop(0))
                for c in in_flight[-1]:
                    c.start()

        def take(i, pc=None):
            copies, now, later = feed[i]
            if copies:
                for c in in_flight.pop(0):
                    c.wait()
                refill(la)
            for work in now:
                work()
            if later:
                pc.spread(later, 0, pw * hm0, tm0)

        refill(3)
        zero[...] = jnp.zeros(zero.shape, zero.dtype)
        for i in range(3 - halves):
            take(i)
        block(0, hm0, tm0, order0, [job(take, i) for i in range(3 - halves, len(feed) - 1)])
        take(len(feed) - 1)

        @pl.loop(0, nb)
        def _(b):
            row = tm0 + b * tm
            block(row, tm // 2, jnp.minimum(row + tm, S - tm), order)

        for part in range(3):
            out_copy(part, 0, hm0).wait()
            for b in range(nb):
                out_copy(part, tm0 + b * tm, tm // 2).wait()

    vm = pltpu.VMEM
    tiles = lambda dtype, *shape: vm(shape + (_L,), dtype)
    return pl.pallas_call(
        kernel,
        in_specs=[pl.BlockSpec(memory_space=pl.ANY)] * 6,
        out_specs=pl.BlockSpec(memory_space=pl.ANY),
        out_shape=jax.ShapeDtypeStruct(A_x.shape, A_x.dtype),
        scratch_shapes=[
            vm((S, D), A_x.dtype), vm((S, D), A_x.dtype), vm((3, D, D), A_wqkv.dtype), vm((D, D), A_wo.dtype),
            vm((F, D), B_w_gate.dtype), vm((F, D), B_w_up.dtype), vm((F, D), B_w_down.dtype),
            [tiles(_F32, ND, D)] * 4, [tiles(_BF16, 16, _L)] * len(pairs), [tiles(_BF16, 16, _L)] * NK,
            tiles(_BF16, ND, _L), tiles(_F32, 2, tm0), tiles(_BF16, 16, tm0 // 2),
            tiles(_F32, ND, tm0), tiles(_F32, ND, tm0 + _HALO), tiles(_F32, ND, tm0 + _HALO),
            tiles(_F32, ND, tm0), tiles(_F32, tm0), tiles(_BF16, 9, NK, tm0 // 2), tiles(_BF16, tm0),
            tiles(jnp.int32, 8), pltpu.SemaphoreType.DMA((3,)), pltpu.SemaphoreType.DMA,
        ],
        compiler_params=pltpu.CompilerParams(vmem_limit_bytes=100 * 1024 * 1024),
        interpret=interpret,
    )(A_x, A_wqkv, A_wo, B_w_gate.T, B_w_up.T, B_w_down)


@jax.jit
def pallas_parallel_sum__sliding_local_dilated__geglu_ffn__prompt_kernel(
    A_x: jax.Array,
    A_wqkv: jax.Array,
    A_wo: jax.Array,
    B_x: jax.Array,
    B_w_gate: jax.Array,
    B_w_up: jax.Array,
    B_w_down: jax.Array,
):
    return _impl(A_x, A_wqkv, A_wo, B_x, B_w_gate, B_w_up, B_w_down)
```

```python
import functools
import math

import jax
import jax.numpy as jnp
from jax import lax
import jax.experimental.pallas as pl
import jax.experimental.pallas.tpu as pltpu

_H, _W, _DIL = 32, 8, 2
_HALO = 16
_L = 128
_F32, _BF16, _U32 = jnp.float32, jnp.bfloat16, jnp.uint32


def _gelu(x):
    c = math.sqrt(2.0 / math.pi)
    hx = 0.5 * x
    return hx + hx * jnp.tanh(x * (c + (c * 0.044715) * (x * x)))


def _lhs7(a11, a12, a21, a22):
    return (a11 + a22, a21 + a22, a11, a22, a11 + a12, a21 - a11, a12 - a22)


def _rhs7(b11, b12, b21, b22):
    return (b11 + b22, b11, b12 - b22, b21 - b11, b22, b11 + b12, b21 + b22)


def _put(ref, idx, r0, v):
    if ref.dtype == _U32:
        ref[idx + (pl.ds(r0 // 2, v.shape[0] // 2),)] = pltpu.bitcast(v.astype(_BF16), _U32)
    else:
        ref[idx + (pl.ds(r0, v.shape[0]),)] = v.astype(_BF16)
    return v[-8:].astype(_F32)


def _get(ref, idx, r0=0, n=_L):
    if ref.dtype == _U32:
        return ref[idx + (pl.ds(r0 // 2, n // 2),)]
    return pltpu.bitcast(ref[idx + (pl.ds(r0, n),)], _U32)


class _Pacer:
    def __init__(self, always):
        self.always, self.now, self.jobs, self.done = always, 0, [], []

    def spread(self, jobs, t0, t1, slack):
        self.jobs += [(self.now + t0 + (t1 - t0) * i // len(jobs), slack, job) for i, job in enumerate(jobs)]
        self.jobs.sort(key=lambda e: e[0])

    def pending(self, fn):
        return sum(job.func is fn for _, _, job in self.jobs)

    def dot(self, lhs, rhs, rhs_transposed):
        due = [v for t, v in self.done if t <= self.now]
        self.done = [(t, v) for t, v in self.done if t > self.now]
        if due:
            head = functools.reduce(lambda u, v: jnp.where(self.always, u, pltpu.bitcast(v, _U32)), due, rhs[0][:8])
            rhs = [jnp.concatenate([head, rhs[0][8:]], axis=0)] + rhs[1:]
        a, b = (jnp.concatenate(v, axis=1) for v in (lhs, rhs))
        a, b = (pltpu.bitcast(v, _BF16) if v.dtype == _U32 else v for v in (a, b))
        r = lax.dot_general(a, b, (((1,), (int(rhs_transposed),)), ((), ())), preferred_element_type=_F32)
        self.now += a.shape[0] * len(lhs) * r.shape[1] // (4 * _L)

        def after(v):
            reps = (v.shape[0] // 8, v.shape[1] // _L)
            return jnp.where(jnp.tile(self.always, reps), v, jnp.tile(r[:8, :_L], reps))

        while self.jobs and self.jobs[0][0] <= self.now:
            _, slack, job = self.jobs.pop(0)
            self.done.append((self.now + slack, job(after)))
        return r


@jax.jit
def pallas_parallel_sum__sliding_local_dilated__geglu_ffn__prompt_kernel(
    A_x: jax.Array,
    A_wqkv: jax.Array,
    A_wo: jax.Array,
    B_x: jax.Array,
    B_w_gate: jax.Array,
    B_w_up: jax.Array,
    B_w_down: jax.Array,
):
    del B_x
    _, S, D = A_x.shape
    F = B_w_gate.shape[1]
    tm0, tm = 512, 256
    nb = (S - tm0) // tm
    Dh = D // _H
    ND, NF = D // _L, F // _L
    FR = F - NF * _L
    assert (ND, NF, FR) == (5, 13, 64) and S == tm0 + nb * tm and nb > 1
    c_exp = Dh ** -0.5 * math.log2(math.e)
    job = functools.partial
    tile = lambda i, n=1: pl.ds(i * _L, n * _L)
    lt = lambda v, j: v[:, j * _L:(j + 1) * _L]
    rows = lambda *parts: jnp.concatenate(parts, axis=0)
    total = lambda parts: functools.reduce(jnp.add, parts)
    qkv = [(kind, j) for kind in "qkv" for j in range(ND)] + [("t", 0)]
    pairs = [(("g", c), ("u", c)) for c in range(NF)] + list(zip(qkv[::2], qkv[1::2]))
    w2_tiles = [("h", c) for c in range(NF)] + [("o", j) for j in range(ND)]
    kpairs = list(zip(w2_tiles[::2], w2_tiles[1::2]))
    NK = len(kpairs)
    stages = {str(i): (2 * i, 2) for i in range(NF // 2)}
    stages.update(h=(NF - 1, 1), A=(NF, 2), B=(NF + 2, 2), C=(NF + 4, 2), V=(NF + 6, 2))
    order0, order = "01hABCV2345", "ABCVh012345"
    seq2 = (0, 3, 4, 2, 1, 6, 5, 7, 8)

    def kernel(x_hbm, wqkv_hbm, wo_hbm, wg_hbm, wu_hbm, wd_hbm, o_hbm,
               x_s, o_s, wqkv_raw, wo_raw, wg_raw, wu_raw, wd_raw, wide, w1, w2, wt,
               stat, xa, q_s, k_s, v_s, att, h_last, zero, i_sem, o_sem):
        def out_copy(part, row, hm):
            r = pl.ds(pl.multiple_of(row + min(part, 1) * hm, 16), hm), (tile(0, 5), tile(0, 4), tile(4))[part]
            return pltpu.make_async_copy(o_s.at[r], o_hbm.at[0].at[r], o_sem)

        def w_rows(kind, t, e):
            if kind in "qkvo":
                return [wide["qkvo".index(kind)][j, pl.ds(4 * t + e, _H, stride=Dh), :] for j in range(ND)]
            if kind == "t":
                ref, r0 = (wg_raw, wu_raw)[e * _H // FR], NF * _L + e * _H % FR
            else:
                ref, r0 = dict(g=wg_raw, u=wu_raw, h=wd_raw)[kind], t * _L + e * _H
            return [ref[pl.ds(r0, _H), tile(j)].astype(_F32) for j in range(ND)]

        def prep_w1(p, e):
            left, right = (w_rows(*t, e) for t in pairs[p])
            for k in range(2):
                for i, b in enumerate(_rhs7(left[k], right[k], left[2 + k], right[2 + k]) + ((left, right)[k][4],)):
                    _put(w1[p], (2 * i + k,), e * _H, b)

        def prep_w2(p, e, after):
            first, second = (w_rows(*t, e) for t in kpairs[p])
            for k in range(2):
                _put(w2[p], (14 + k,), e * _H, (first, second)[k][4])
                for i, b in enumerate(_rhs7(after(first[k]), first[2 + k], second[k], after(second[2 + k]))):
                    out = _put(w2[p], (2 * i + k,), e * _H, b)
            return out

        def widen_wo(j, after):
            wide[3][j] = wo_raw[:, tile(j)].astype(_F32)
            _put(wt, (j,), FR, jnp.zeros((_L - FR, _L), _F32))
            return _put(wt, (j,), 0, wd_raw[pl.ds(NF * _L, FR), tile(j)])

        def transpose_qkv(s, j):
            wide[s][j] = wqkv_raw[s, tile(j), :].astype(_F32).T

        def row_stats(row, r, n, after=lambda v: v):
            x = after(x_s[pl.ds(pl.multiple_of(row + r, 16), n), :].astype(_F32))
            mean = jnp.mean(x, axis=-1, keepdims=True)
            xc = x - mean
            scale = jnp.broadcast_to(lax.rsqrt(jnp.mean(xc * xc, axis=-1, keepdims=True) + 1e-5), (n, _L))
            stat[0, pl.ds(r, n), :] = jnp.broadcast_to(mean, (n, _L))
            stat[1, pl.ds(r, n), :] = scale
            return scale[-8:]

        def normalize(row, hm, r, n, after=lambda v: v):
            xn = []
            for r0 in (r, hm + r):
                mean, scale = after(stat[0, pl.ds(r0, n), :]), stat[1, pl.ds(r0, n), :]
                x = x_s[pl.ds(pl.multiple_of(row + r0, 16), n), :].astype(_F32)
                xn.append([(lt(x, j) - mean) * scale for j in range(ND)])
            for k in range(2):
                _put(xa, (14 + k,), r, xn[k][4])
                for i, a in enumerate(_lhs7(xn[0][k], xn[0][2 + k], xn[1][k], xn[1][2 + k])):
                    out = _put(xa, (2 * i + k,), r, a)
            return out

        def project(pc, c, n, r0, nr, midway):
            a = lambda i: [_get(xa, (2 * i + k,), r0, nr) for k in range(2)]
            b = lambda i, ps: [rows(*[_get(w1[p], (2 * i + k,)) for p in ps]) for k in range(2)]
            m = [pc.dot(a(i), b(i, range(c, c + n)), True) for i in range(5)]
            midway(pc)
            out = []
            for p in range(c, c + n):
                e = [lt(m[i], p - c) for i in range(5)]
                (top, bot), (left, right) = a(7), b(7, [p])
                c11 = pc.dot(a(6) + [top], b(6, [p]) + [left], True) + (e[0] + e[3] - e[4])
                c12 = pc.dot([top], [right], True) + (e[2] + e[4])
                c22 = pc.dot(a(5) + [bot], b(5, [p]) + [right], True) + (e[0] - e[1] + e[2])
                c21 = pc.dot([bot], [left], True) + (e[1] + e[3])
                out.append((c11, c12, c21, c22))
            return out

        left2 = {}

        def put_h(p, a11, a12, a21, a22):
            for i, a in enumerate(_lhs7(a11, a12, a21, a22) + (a12, a21)):
                left2.setdefault((i, p), []).append(a.astype(_BF16))
            return a11[-8:]

        def stage(pc, name, r0, nr, midway):
            c, n = stages[name]
            res = project(pc, c, n, r0, nr, midway)
            if c < NF:
                h = [(_gelu(gt) * ut, _gelu(gb) * ub) for gt, ut, gb, ub in res]
                if n == 2:
                    put_h(c // 2, h[0][0], h[1][0], h[0][1], h[1][1])
                else:
                    h_last[pl.ds(0, 2 * nr), :] = rows(*h[0])
                return
            for pair, quad in zip(pairs[c:c + n], res):
                for side, (kind, j) in enumerate(pair):
                    r = rows(*quad[side::2])
                    if kind == "t":
                        lane = lax.broadcasted_iota(jnp.int32, r.shape, 1)
                        left2["t"] = jnp.where(lane < FR, _gelu(r) * pltpu.roll(r, FR, 1), 0.0)
                    else:
                        dict(q=q_s, k=k_s, v=v_s)[kind][j, pl.ds(0 if kind == "q" else _HALO, 2 * nr), :] = r

        def attention(r0, first, after):
            back = lambda ref, j, w: ref[j, pl.ds(r0 + _HALO - _DIL * w, 8), :]
            q = [after(q_s[j, pl.ds(r0, 8), :]) for j in range(ND)]
            logits = []
            for w in range(_W):
                a = total([q[j] * back(k_s, j, w) for j in range(ND)])
                a = (a + pltpu.roll(a, 2 * _H, 1)) + (pltpu.roll(a, _H, 1) + pltpu.roll(a, 3 * _H, 1))
                if first and r0 < _DIL * w:
                    pos = r0 + lax.broadcasted_iota(jnp.int32, a.shape, 0)
                    a = jnp.where(pos >= _DIL * w, a, -1e9 * Dh ** 0.5)
                logits.append(a)
            m = functools.reduce(jnp.maximum, logits)
            p = [jnp.exp2((a - m) * c_exp) for a in logits]
            inv = 1.0 / total(p)
            for j in range(ND):
                o = inv * total([p[w] * back(v_s, j, w) for w in range(_W)])
                att[j, pl.ds(r0, 8), :] = o
            return o

        def pack_attention(r, hm, after):
            t = lambda i, r0: att[i - 1, pl.ds(r0, 16), :] if i else h_last[pl.ds(r0, 16), :]
            return [put_h(NF // 2 + i // 2, t(i, r), t(i + 1, r), t(i, hm + r), t(i + 1, hm + r))
                    for i in range(0, ND + 1, 2)][-1]

        def output(pc, row, hm):
            a = lambda i, ps: [rows(*left2[i, p]) for p in ps]
            bt = lambda j, n: [_get(wt, (j + k,)) for k in range(n)]
            top, bot = left2["t"][:hm].astype(_BF16), left2["t"][hm:].astype(_BF16)

            def emit(half, j, y):
                r = pl.ds(pl.multiple_of(row + half * hm, 16), hm), pl.ds(j * _L, y.shape[1])
                o_s[r] = (x_s[r].astype(_F32) + y).astype(o_s.dtype)

            def product(i, ps, extra=()):
                if i < 7:
                    lhs, rhs = a(i, ps), [rows(*[_get(w2[p], (2 * i + k,)) for p in ps]) for k in range(2)]
                else:
                    lhs = [v for p in ps for j in ((2, 7), (8, 3))[i - 7] for v in a(j, [p])]
                    rhs = [rows(*[_get(w2[p], (k,)) for p in ps for k in (14, 15)])]
                if extra:
                    lhs, rhs = lhs + [extra[0]], list(map(rows, rhs, extra[1]))
                return pc.dot(lhs, rhs, False)

            assert not pc.pending(prep_w2)
            ffn = {i: [product(i, range(p, p + 2)) for p in range(0, NF // 2, 2)] for i in seq2}
            assert len(pc.jobs) == pc.pending(normalize)
            k_s[:, pl.ds(0, _HALO), :] = k_s[:, pl.ds(2 * hm, _HALO), :]
            v_s[:, pl.ds(0, _HALO), :] = v_s[:, pl.ds(2 * hm, _HALO), :]
            full = lambda i, *extra: total(ffn[i] + [product(i, range(NF // 2, NK), extra)])
            m = {i: full(i) for i in seq2[:5]}
            emit(0, 2, pc.dot([top], bt(2, 2), False) + (m[2] + m[4]))
            emit(0, 0, full(6, top, bt(0, 2)) + (m[0] + m[3] - m[4]))
            emit(0, 4, full(7, top, bt(4, 1)))
            out_copy(0, row, hm).start()
            emit(1, 0, pc.dot([bot], bt(0, 2), False) + (m[1] + m[3]))
            emit(1, 2, full(5, bot, bt(2, 2)) + (m[0] - m[1] + m[2]))
            out_copy(1, row, hm).start()
            emit(1, 4, full(8, bot, bt(4, 1)))
            out_copy(2, row, hm).start()

        def block(row, hm, next_row, names, hooks=None):
            first = hooks is not None
            left2.clear()
            pc = _Pacer(zero[...] == 0)
            stats = [job(row_stats, next_row, r, 16) for r in range(0, tm, 16)]
            pc.spread(stats, (30 if first else 0) * hm, (58 if first else 36) * hm, 500)
            for i, name in enumerate(names):
                nr = hm // 2 if first and i == 0 else hm
                for r0 in range(0, hm, nr):
                    stage(pc, name, r0, nr, hooks.pop(0) if first else lambda pc: None)
                if name == "V":
                    if first:
                        k_s[:, pl.ds(0, _HALO), :] = jnp.zeros((ND, _HALO, _L), _F32)
                        for j in range(ND):
                            v_s[j, pl.ds(0, _HALO), :] = jnp.broadcast_to(v_s[j, pl.ds(_HALO, 1), :], (_HALO, _L))
                    jobs = []
                    for r in range(0, hm, 16):
                        jobs += [job(attention, r + s, first) for s in (0, 8, hm, hm + 8)]
                        jobs.append(job(pack_attention, r, hm))
                    pc.spread(jobs, 0, (61 if first else 78) * hm, 600)
                if name == "h" and "V" in names[:i]:
                    assert pc.pending(pack_attention) == hm // 16
            assert not pc.pending(row_stats)
            pc.spread([job(normalize, next_row, tm // 2, r, 16) for r in range(0, tm // 2, 16)], 26 * hm, 39 * hm, 300)
            output(pc, row, hm)
            assert not pc.jobs

        feed = [([], [], []) for _ in range(len(order0) + 3)]
        by_rows = lambda src, dst, r0, n: (src.at[pl.ds(r0, n)], dst.at[pl.ds(r0, n)])
        wait_at = lambda i: feed[2 + max(j for j in (0, 1, 2, 3, 4, 6, 8, 10) if j <= i)][0]
        hm0, xr = tm0 // 2, tm0 // 4
        for i in range(2):
            feed[i][0].extend(by_rows(x_hbm.at[0], x_s, r0, xr) for r0 in (i * xr, hm0 + i * xr))
            feed[i][1].extend([job(row_stats, 0, i * xr, xr), job(row_stats, 0, hm0 + i * xr, xr),
                               job(normalize, 0, hm0, i * xr, xr)])
        for s in range(3):
            wait_at(2 + s).append((wqkv_hbm.at[:, pl.ds(s * D, D)], wqkv_raw.at[s]))
            feed[4 + s][1].extend(job(transpose_qkv, s, j) for j in range(ND))
        for i, name in enumerate(order0):
            c, n = stages[name]
            if c < NF or name == "V":
                r0, nr = (c * _L, n * _L) if c < NF else (NF * _L, FR)
                wait_at(i).extend([by_rows(wg_hbm, wg_raw, r0, nr), by_rows(wu_hbm, wu_raw, r0, nr)])
            feed[2 + i][1].extend(job(prep_w1, p, e) for p in range(c, c + n) for e in range(4))
        for i, (lo, hi) in zip((6, 6, 8, 10), ((0, 2), (2, 4), (4, 6), (6, NK))):
            wait_at(i).append(by_rows(wd_hbm, wd_raw, 2 * lo * _L, min(F, 2 * hi * _L) - 2 * lo * _L))
            if hi == NK:
                wait_at(i).append((wo_hbm, wo_raw))
                feed[2 + i][2].extend(job(widen_wo, j) for j in range(ND))
            feed[2 + i][2].extend(job(prep_w2, p, e) for p in range(lo, hi) for e in range(4))
        wait_at(4).append(by_rows(x_hbm.at[0], x_s, tm0, tm))
        feed.append(([by_rows(x_hbm.at[0], x_s, tm0 + tm, S - tm0 - tm)], [], []))
        feed[1:3] = feed[2], feed[1]
        queue = [f[0] for f in feed if f[0]]
        for i, group in enumerate(queue):
            group[:] = [pltpu.make_async_copy(src, dst, i_sem.at[i % 3]) for src, dst in group]
        in_flight = []

        def refill():
            while queue and len(in_flight) < (3 if len(queue) > 1 else 1):
                in_flight.append(queue.pop(0))
                for c in in_flight[-1]:
                    c.start()

        def take(i, pc=None):
            copies, now, later = feed[i]
            assert copies is not wait_at(4) or pc.pending(row_stats) == tm // 16
            if copies:
                for c in in_flight.pop(0):
                    c.wait()
                refill()
            for work in now:
                work()
            if later:
                pc.spread(later, 0, 12 * hm0, tm0)

        refill()
        zero[...] = jnp.zeros(zero.shape, zero.dtype)
        take(0)
        take(1)
        block(0, hm0, tm0, order0, [job(take, i) for i in range(2, len(feed) - 1)])
        take(len(feed) - 1)

        @pl.loop(0, nb)
        def _(b):
            row = tm0 + b * tm
            block(row, tm // 2, jnp.minimum(row + tm, S - tm), order)

        pltpu.make_async_copy(o_s, o_hbm.at[0], o_sem).wait()

    vm = pltpu.VMEM
    tiles = lambda dtype, *shape: vm(shape[:-1] + (shape[-1] // (1 + (dtype == _U32)), _L), dtype)
    return pl.pallas_call(
        kernel,
        in_specs=[pl.BlockSpec(memory_space=pl.ANY)] * 6,
        out_specs=pl.BlockSpec(memory_space=pl.ANY),
        out_shape=jax.ShapeDtypeStruct(A_x.shape, A_x.dtype),
        scratch_shapes=[
            vm((S, D), A_x.dtype), vm((S, D), A_x.dtype), vm((3, D, D), A_wqkv.dtype), vm((D, D), A_wo.dtype),
            vm((F, D), B_w_gate.dtype), vm((F, D), B_w_up.dtype), vm((F, D), B_w_down.dtype),
            [tiles(_F32, ND, D)] * 4, [tiles(_U32, 16, _L)] * len(pairs), [tiles(_BF16, 16, _L)] * NK,
            tiles(_BF16, ND, _L), tiles(_F32, 2, tm0), tiles(_U32, 16, tm0 // 2),
            tiles(_F32, ND, tm0), tiles(_F32, ND, tm0 + _HALO), tiles(_F32, ND, tm0 + _HALO),
            tiles(_F32, ND, tm0), tiles(_F32, tm0),
            tiles(jnp.int32, 8), pltpu.SemaphoreType.DMA((3,)), pltpu.SemaphoreType.DMA,
        ],
        compiler_params=pltpu.CompilerParams(vmem_limit_bytes=100 * 1024 * 1024),
    )(A_x, A_wqkv, A_wo, B_w_gate.T, B_w_up.T, B_w_down)
```
